```python
import jax
import jax.numpy as jnp

def _softmax(x, axis=-1):
    return jax.nn.softmax(x, axis=axis)

def _gelu(x):
    return jax.nn.gelu(x, approximate=True)

def _silu(x):
    return jax.nn.silu(x)

def _sigmoid(x):
    return jax.nn.sigmoid(x)

def _layernorm(x, axis=-1, eps=1e-05):
    m = jnp.mean(x, axis=axis, keepdims=True)
    v = jnp.var(x, axis=axis, keepdims=True)
    return (x - m) / jnp.sqrt(v + eps)

def _scatter_add(tgt, idx, src, axis=0):
    return tgt.at[idx].add(src)

def _segment_sum(src, seg, n):
    return jax.ops.segment_sum(src, seg, n)

class _Rng:

    def __init__(self, key):
        self._k = key

    def _next(self):
        self._k, sub = jax.random.split(self._k)
        return sub

    def normal(self, shape):
        return jax.random.normal(self._next(), shape, dtype=jnp.bfloat16)

    def randint(self, lo, hi, shape):
        return jax.random.randint(self._next(), shape, lo, hi, dtype=jnp.int32)

    def uniform(self, shape, lo=0.0, hi=1.0):
        return jax.random.uniform(self._next(), shape, jnp.bfloat16, lo, hi)

    def permutation(self, n):
        return jax.random.permutation(self._next(), n)
kernel_name = 'adaLN_cond__sliding_local_dilated__mixer_s_mlp__prompt'

def setup_inputs():
    _rng = _Rng(jax.random.key(int.from_bytes(__import__("os").urandom(4), "little")))
    _w = lambda a: (lambda t: t.astype(jnp.bfloat16) if jnp.issubdtype(t.dtype, jnp.floating) else t)(jnp.asarray(a))

    def _A_setup():
        B, S, D = (1, 2048, 1024)
        return {'x': _w((lambda *s: _rng.normal(s) * 0.05)(B, S, D)), 'wqkv': _w((lambda *s: _rng.normal(s) * 0.05)(D, 3 * D)), 'wo': _w((lambda *s: _rng.normal(s) * 0.05)(D, D))}
    _A_in = _A_setup()

    def _B_setup():
        B, S, D, F = (1, 2048, 1024, 3584)
        return {'x': _w((lambda *s: _rng.normal(s) * 0.05)(B, S, D)), 'w1': _w((lambda *s: _rng.normal(s) * 0.05)(D, D) * D ** (-0.5)), 'w2': _w((lambda *s: _rng.normal(s) * 0.05)(D, D) * D ** (-0.5)), 'w3': _w((lambda *s: _rng.normal(s) * 0.05)(D, F) * D ** (-0.5)), 'w4': _w((lambda *s: _rng.normal(s) * 0.05)(F, D) * F ** (-0.5))}
    _B_in = _B_setup()
    return {'A_x': _A_in['x'], 'A_wqkv': _A_in['wqkv'], 'A_wo': _A_in['wo'], 'B_x': _B_in['x'], 'B_w1': _B_in['w1'], 'B_w2': _B_in['w2'], 'B_w3': _B_in['w3'], 'B_w4': _B_in['w4'], 'c': _w((lambda *s: _rng.normal(s) * 0.05)(1, 1024)), 'w_mod': _w((lambda *s: _rng.normal(s) * 0.05)(1024, 6 * 1024) * 1024 ** (-0.5))}

def reference(A_x, A_wqkv, A_wo, B_x, B_w1, B_w2, B_w3, B_w4, c, w_mod):

    def _A_ref(x, wqkv, wo):
        B, S, D = x.shape
        H = 32
        Dh = D // H
        W, dil = (8, 2)
        qkv = (lambda x, *d: x.transpose(*d))((x @ wqkv).reshape(B, S, 3, H, Dh), 2, 0, 3, 1, 4)
        q, k, v = (qkv[0], qkv[1], qkv[2])
        scale = Dh ** (-0.5)
        pos = jnp.arange(S)
        off = jnp.arange(W) * dil
        idx = pos[:, None] - off[None, :]
        mask = idx >= 0
        idx_c = jnp.where(mask, idx, 0).reshape(-1)
        kg = k[:, :, idx_c, :].reshape(B, H, S, W, Dh)
        vg = v[:, :, idx_c, :].reshape(B, H, S, W, Dh)
        logits = jnp.einsum('bhsd,bhswd->bhsw', q, kg) * scale
        logits = jnp.where(mask[None, None, :, :], logits, -1000000000.0)
        attn = _softmax(logits, axis=-1)
        o = jnp.einsum('bhsw,bhswd->bhsd', attn, vg)
        return (lambda x, *d: x.transpose(*d))(o, 0, 2, 1, 3).reshape(B, S, D) @ wo

    def _B_ref(x, w1, w2, w3, w4):
        B, S, D = x.shape
        h = _gelu(_layernorm(x, axis=-1) @ w1)
        c = D // 4
        g0 = jnp.pad(h[:, :, 0 * c:1 * c], ((0, 0), (1, 0), (0, 0)))[:, :S, :]
        g1 = jnp.pad(h[:, :, 1 * c:2 * c], ((0, 0), (0, 1), (0, 0)))[:, 1:, :]
        g2 = jnp.pad(h[:, :, 2 * c:3 * c], ((0, 0), (2, 0), (0, 0)))[:, :S, :]
        g3 = jnp.pad(h[:, :, 3 * c:], ((0, 0), (0, 2), (0, 0)))[:, 2:, :]
        hs = jnp.concatenate([g0, g1, g2, g3], axis=-1) @ w2
        x1 = x + hs
        h2 = _gelu(_layernorm(x1, axis=-1) @ w3) @ w4
        return x1 + h2
    x = A_x
    mod = (_silu(c) @ w_mod).reshape(c.shape[0], 6, 1, -1)
    sa, ca, ga, sb, cb, gb = (mod[:, 0].copy(), mod[:, 1].copy(), mod[:, 2].copy(), mod[:, 3].copy(), mod[:, 4].copy(), mod[:, 5].copy())
    h = _layernorm(x, axis=-1) * (1 + ca) + sa
    x = x + ga * _A_ref(h, A_wqkv, A_wo)
    h = _layernorm(x, axis=-1) * (1 + cb) + sb
    x = x + gb * _B_ref(h, B_w1, B_w2, B_w3, B_w4)
    return x
```

```python
import jax
import jax.numpy as jnp
import jax.experimental.pallas as pl
import jax.experimental.pallas.tpu as pltpu

S, D, F = 2048, 1024, 3584
P = 16
NP = 4
TM = NP * 128
FC = 512
NQ = 2
TQ = NQ * 128
f32, bf16 = jnp.float32, jnp.bfloat16


def _ln(x):
    xc = x - jnp.mean(x, axis=-1, keepdims=True)
    return xc * jax.lax.rsqrt(jnp.mean(xc * xc, axis=-1, keepdims=True) + 1e-5)


def _dot(a, b):
    return jnp.dot(a, b, preferred_element_type=f32)


def _kernel(c_ref, x_h, wqkv_h, wo_h, w1_h, w2_h, w3_h, w4_h, wm_h, o_ref,
            xb, wqkv, wo, w1, w2, w3, w4, wm, xs, xp, hp, qT, kT, vT, g, sems):
    srcs = [x_h, wm_h.at[:, 0:2048], wqkv_h.at[:, 0:D], wm_h.at[:, 2048:], wo_h, w1_h, w2_h, w3_h, w4_h, wqkv_h.at[:, D:]]
    dsts = [xb, wm.at[:, 0:2048], wqkv.at[:, 0:D], wm.at[:, 2048:], wo, w1, w2, w3, w4, wqkv.at[:, D:]]
    cps = [pltpu.make_async_copy(s, d, sems.at[i]) for i, (s, d) in enumerate(zip(srcs, dsts))]
    for i in (0, 1, 2, 9, 3, 4, 5, 6, 7, 8):
        cps[i].start()
    cv = jnp.broadcast_to(c_ref[...].astype(f32), (8, D))
    sc = (cv * jax.nn.sigmoid(cv)).astype(bf16)
    cps[0].wait()
    for j in range(8):
        xs[j] = xb[:, j * 128:(j + 1) * 128].astype(f32)

    @pl.loop(0, P)
    def _(p):
        r = pl.ds(pl.multiple_of(p * 128, 128), 128)
        for j in range(8):
            xp[r, j * 128:(j + 1) * 128] = xs[j, pl.ds(p, 128, stride=P), :]
        hp[r, :] = _ln(xp[r, :])

    cps[1].wait()
    m0 = _dot(sc, wm[:, 0:2048])[0:1]
    sa, ca1 = m0[:, :D], 1.0 + m0[:, D:]
    cps[2].wait()

    def proj(t, ns):
        r = pl.ds(pl.multiple_of(t * TM, TM), TM)
        h = (hp[r, :] * ca1 + sa).astype(bf16)
        for n, dst in ns:
            y = _dot(h, wqkv[:, n * D:(n + 1) * D])
            if n == 0:
                y = y * (32 ** -0.5)
            for i in range(NP):
                p = t * NP + i
                yt = y[i * 128:(i + 1) * 128].T
                if n == 0:
                    dst[p] = yt
                else:
                    dst[p + P] = yt
                    dst[p] = pltpu.roll(yt, 1, 1)

    pl.loop(0, P // NP)(lambda t: proj(t, ((0, qT),)))
    cps[9].wait()
    pl.loop(0, P // NP)(lambda t: proj(t, ((1, kT), (2, vT))))
    cps[3].wait()
    m1 = _dot(sc, wm[:, 2048:])[0:1]
    ga, sb, cb1, gb = m1[:, :D], m1[:, D:2 * D], 1.0 + m1[:, 2 * D:3 * D], m1[:, 3 * D:]
    cps[4].wait()
    cps[5].wait()
    lane = jax.lax.broadcasted_iota(jnp.int32, (8, 128), 1)
    row = jax.lax.broadcasted_iota(jnp.int32, (128, D), 0)

    def attn(p):
        outs = []
        for h in range(32):
            hs = slice(h * 32, h * 32 + 32)
            q = qT[p, hs, :]
            lg = []
            for w in range(8):
                pr = q * kT[p + P - 2 * w, hs, :]
                s = (pr[0:8] + pr[8:16]) + (pr[16:24] + pr[24:32])
                s = s + pltpu.roll(s, 4, 0)
                s = s + pltpu.roll(s, 2, 0)
                s = s + pltpu.roll(s, 1, 0)
                if w:
                    s = jnp.where((lane == 0) & (p < 2 * w), -1e9, s)
                lg.append(s)
            mx = lg[0]
            for s in lg[1:]:
                mx = jnp.maximum(mx, s)
            e = [jnp.exp(s - mx) for s in lg]
            den = e[0]
            for s in e[1:]:
                den = den + s
            inv = 1.0 / den
            v = vT[p + P, hs, :]
            acc = [e[0] * v[i * 8:i * 8 + 8] for i in range(4)]
            for w in range(1, 8):
                v = vT[p + P - 2 * w, hs, :]
                acc = [acc[i] + e[w] * v[i * 8:i * 8 + 8] for i in range(4)]
            outs += [a * inv for a in acc]
        return jnp.concatenate(outs, axis=0).T.astype(bf16)

    def attn_tile(t):
        for i in range(NP):
            xb[pl.ds(pl.multiple_of(t * TM + i * 128, 128), 128), :] = attn(t * NP + i)

    def mid(t):
        r = pl.ds(pl.multiple_of(t * TM, TM), TM)
        o = xb[r, :]
        x1 = xp[r, :] + ga * _dot(o, wo[...])
        xp[r, :] = x1
        h = _ln(x1) * cb1 + sb
        hp[r, :] = h
        y = jax.nn.gelu(_dot(_ln(h).astype(bf16), w1[...]), approximate=True)
        for i in range(NP):
            g[t * NP + i + 2] = y[i * 128:(i + 1) * 128].astype(bf16)

    @pl.loop(0, P)
    def _(p):
        xb[pl.ds(pl.multiple_of(p * 128, 128), 128), :] = attn(p)

    pl.loop(0, P // NP)(mid)
    for i in range(2):
        g[i] = jnp.where(row == 0, 0.0, pltpu.roll(g[P + i].astype(f32), 1, 0)).astype(bf16)
        g[P + 2 + i] = jnp.where(row == 127, 0.0, pltpu.roll(g[2 + i].astype(f32), 127, 0)).astype(bf16)
    cps[6].wait()
    cps[7].wait()
    cps[8].wait()

    @pl.loop(0, P // NQ)
    def _(t):
        r = pl.ds(pl.multiple_of(t * TQ, TQ), TQ)
        gs = jnp.concatenate([jnp.concatenate(
            [g[t * NQ + i + 2 + sh, :, k * 256:(k + 1) * 256] for k, sh in enumerate((-1, 1, -2, 2))],
            axis=1) for i in range(NQ)], axis=0)
        acc = hp[r, :] + _dot(gs, w2[...])
        hb = _ln(acc).astype(bf16)
        for f in range(F // FC):
            fs = slice(f * FC, (f + 1) * FC)
            u = jax.nn.gelu(_dot(hb, w3[:, fs]), approximate=True).astype(bf16)
            acc = acc + _dot(u, w4[fs, :])
        out = xp[r, :] + gb * acc
        for i in range(NQ):
            for j in range(8):
                xs[j, pl.ds(t * NQ + i, 128, stride=P), :] = out[i * 128:(i + 1) * 128, j * 128:(j + 1) * 128]

    for j in range(8):
        o_ref[:, j * 128:(j + 1) * 128] = xs[j].astype(bf16)


@jax.jit
def pallas_adaLN_cond__sliding_local_dilated__mixer_s_mlp__prompt_kernel(
        A_x, A_wqkv, A_wo, B_x, B_w1, B_w2, B_w3, B_w4, c, w_mod):
    any_ = pl.BlockSpec(memory_space=pl.ANY)
    vm = pl.BlockSpec(memory_space=pltpu.VMEM)
    V = pltpu.VMEM
    out = pl.pallas_call(
        _kernel,
        out_shape=jax.ShapeDtypeStruct((S, D), bf16),
        in_specs=[vm] + [any_] * 8,
        out_specs=vm,
        scratch_shapes=[V((S, D), bf16), V((D, 3 * D), bf16), V((D, D), bf16), V((D, D), bf16),
                        V((D, D), bf16), V((D, F), bf16), V((F, D), bf16), V((D, 6 * D), bf16),
                        V((8, S, 128), f32), V((S, D), f32), V((S, D), f32),
                        V((P, D, 128), f32), V((2 * P, D, 128), f32), V((2 * P, D, 128), f32),
                        V((P + 4, 128, D), bf16), pltpu.SemaphoreType.DMA((10,))],
        compiler_params=pltpu.CompilerParams(vmem_limit_bytes=126 * 1024 * 1024),
    )(c, A_x.reshape(S, D), A_wqkv, A_wo, B_w1, B_w2, B_w3, B_w4, w_mod)
    return out.reshape(1, S, D)
```
